```python
import os as _os
_os.environ.setdefault("JAX_PLATFORMS", "cpu")
import jax
import jax.numpy as jnp

def _softmax(x, axis=-1):
    return jax.nn.softmax(x, axis=axis)
def _gelu(x):
    return jax.nn.gelu(x, approximate=True)
def _silu(x):
    return jax.nn.silu(x)
def _sigmoid(x):
    return jax.nn.sigmoid(x)
def _layernorm(x, axis=-1, eps=1e-5):
    m = jnp.mean(x, axis=axis, keepdims=True)
    v = jnp.var(x, axis=axis, keepdims=True)
    return (x - m) / jnp.sqrt(v + eps)
def _scatter_add(tgt, idx, src, axis=0):
    return tgt.at[idx].add(src)
def _segment_sum(src, seg, n):
    return jax.ops.segment_sum(src, seg, n)
class _Rng:
    def __init__(self, key):
        self._k = key
    def _next(self):
        self._k, sub = jax.random.split(self._k)
        return sub
    def normal(self, shape):
        return jax.random.normal(self._next(), shape, dtype=jnp.bfloat16)
    def randint(self, lo, hi, shape):
        return jax.random.randint(self._next(), shape, lo, hi, dtype=jnp.int32)
    def uniform(self, shape, lo=0.0, hi=1.0):
        return jax.random.uniform(self._next(), shape, jnp.bfloat16, lo, hi)
    def permutation(self, n):
        return jax.random.permutation(self._next(), n)


kernel_name = 'concat_heads__grouped_kv_mqa__sliding_block__prompt'

def setup_inputs():
    _rng = _Rng(jax.random.key(int.from_bytes(__import__("os").urandom(4), "little")))
    _w = (lambda a: (lambda t: t.astype(jnp.bfloat16) if jnp.issubdtype(t.dtype, jnp.floating) else t)(jnp.asarray(a)))
    def _A_setup():
        B, S, D, H = 1, 2048, 1024, 32
        Dh = D // H
        return {
            "x": _w((lambda *s: _rng.normal(s) * 0.05)(B, S, D)),
            "wq": _w((lambda *s: _rng.normal(s) * 1.6)(D, H * Dh)),
            "wk": _w((lambda *s: _rng.normal(s) * 1.6)(D, Dh)),
            "wv": _w((lambda *s: _rng.normal(s) * 0.1)(D, Dh)),
            "wo": _w((lambda *s: _rng.normal(s) * 0.1)(H * Dh, D)),
        }
    _A_in = _A_setup()

    def _B_setup():
        B, S, D = 1, 2048, 1024
        return {
            "x": _w((lambda *s: _rng.normal(s) * 0.2)(B, S, D)),
            "wqkv": _w((lambda *s: _rng.normal(s) * 0.2)(D, 3 * D)),
            "wo": _w((lambda *s: _rng.normal(s) * 0.05)(D, D)),
        }
    _B_in = _B_setup()

    return {
        "A_x": _A_in["x"],
        "A_wq": _A_in["wq"],
        "A_wk": _A_in["wk"],
        "A_wv": _A_in["wv"],
        "A_wo": _A_in["wo"],
        "B_x": _B_in["x"],
        "B_wqkv": _B_in["wqkv"],
        "B_wo": _B_in["wo"],
    }

def reference(A_x, A_wq, A_wk, A_wv, A_wo, B_x, B_wqkv, B_wo):
    def _A_ref(x, wq, wk, wv, wo):
        B, S, D = x.shape
        H = 32
        Dh = D // H
        q = (lambda x, *d: x.transpose(*d))((x @ wq).reshape(B, S, H, Dh), 0, 2, 1, 3)
        k = x @ wk
        v = x @ wv
        scores = jnp.einsum("bhqd,bkd->bhqk", q, k) * (Dh ** -0.5)
        p = _softmax(scores, axis=-1)
        o = jnp.einsum("bhqk,bkd->bhqd", p, v)
        return (lambda x, *d: x.transpose(*d))(o, 0, 2, 1, 3).reshape(B, S, H * Dh) @ wo

    def _B_ref(x, wqkv, wo):
        B, S, D = x.shape
        H = 32; Dh = D // H; W = 256
        qkv = (lambda x, *d: x.transpose(*d))((x @ wqkv).reshape(B, S, 3, H, Dh), 2, 0, 3, 1, 4)
        q, k, v = qkv[0], qkv[1], qkv[2]
        scores = jnp.einsum("bhqd,bhkd->bhqk", q, k) * (Dh ** -0.5)
        idx = jnp.arange(S)
        mask = (idx[:, None] - idx[None, :] >= 0) & (idx[:, None] - idx[None, :] < W)
        scores = jnp.where(mask[None, None], scores, -1e9)
        p = _softmax(scores, axis=-1)
        o = jnp.einsum("bhqk,bhkd->bhqd", p, v)
        return (lambda x, *d: x.transpose(*d))(o, 0, 2, 1, 3).reshape(B, S, D) @ wo

    a = _A_ref(A_x, A_wq, A_wk, A_wv, A_wo)
    b = _B_ref(B_x, B_wqkv, B_wo)
    return jnp.concatenate([a, b], axis=-1)
```

```python
import functools
import jax, jax.numpy as jnp
from jax import lax
from jax.experimental import pallas as pl
from jax.experimental.pallas import tpu as pltpu

S = 2048; D = 1024; H = 32; DH = 32; W = 256
LOG2E = 1.4426950408889634
SCALE = (DH ** -0.5) * LOG2E
f32 = jnp.float32; bf16 = jnp.bfloat16
NEG = -1e30
RC = 512
NRC = S // RC
CB = 512; KC = 128
QB = 128; NG = H // 4; NQ = S // QB
CH = (2, 1, 0)

def dot_tt(w, x): return lax.dot_general(w, x, (((0,), (1,)), ((), ())), preferred_element_type=f32)
def dot_nt(a, b): return lax.dot_general(a, b, (((1,), (1,)), ((), ())), preferred_element_type=f32)
def dot_tn(a, b): return lax.dot_general(a, b, (((0,), (0,)), ((), ())), preferred_element_type=f32)
def dot_nn(a, b): return jnp.dot(a, b, preferred_element_type=f32)

def _make():
    def kernel(ax_hbm, wq_hbm, wkt_hbm, wvt_hbm, awo_hbm, bx_hbm, wqkv_hbm, bwo_hbm, out_hbm,
               xa, wq, wkt, wvt, awo, xb, wqkv, bwo,
               ka, vta, qta, ota, qbd, kb, vtb, otb, s_ref, outv, isem, osem):
        def cp(src, dst, i): return pltpu.make_async_copy(src, dst, isem.at[i])
        c_wk = cp(wkt_hbm, wkt, 0); c_wv = cp(wvt_hbm, wvt, 1); c_wq = cp(wq_hbm, wq, 2)
        c_xa = [cp(ax_hbm.at[pl.ds(c * RC, RC), :], xa.at[pl.ds(c * RC, RC), :], 3 + c) for c in range(NRC)]
        c_awo = cp(awo_hbm, awo, 7); c_wqkv = cp(wqkv_hbm, wqkv, 8); c_xb = cp(bx_hbm, xb, 9); c_bwo = cp(bwo_hbm, bwo, 10)
        c_wk.start(); c_wv.start(); c_xa[0].start(); c_wq.start()
        for c in range(1, NRC): c_xa[c].start()
        def zbody(i, carry):
            qbd[pl.ds(pl.multiple_of(i * 128, 128), 128), :] = jnp.zeros((128, 4 * S), bf16)
            return carry
        lax.fori_loop(0, D // 128, zbody, 0)
        vtb[:, 0:W] = jnp.zeros((D, W), bf16)
        kb[0:W, :] = jnp.zeros((W, D), bf16)
        c_wk.wait(); c_wv.wait()
        for c in range(NRC):
            c_xa[c].wait()
            if c == 0:
                c_wq.wait()
                c_wqkv.start(); c_xb.start(); c_awo.start(); c_bwo.start()
            x = xa[c*RC:(c+1)*RC, :]
            ka[c*RC:(c+1)*RC, :] = dot_nt(x, wkt[...]).astype(bf16)
            vta[:, c*RC:(c+1)*RC] = dot_nt(wvt[...], x).astype(bf16)
            qta[:, c*RC:(c+1)*RC] = (dot_tt(wq[...], x) * SCALE).astype(bf16)

        nqb = S // CB; nch = S // KC; nblk = H * nqb
        def a_idx(j):
            return pl.multiple_of((j // nqb) * DH, DH), pl.multiple_of((j % nqb) * CB, CB)
        def a_qk(j, c, slot):
            r0, c0 = a_idx(j)
            s_ref[slot] = dot_nn(ka[c*KC:(c+1)*KC, :], qta[pl.ds(r0, DH), pl.ds(c0, CB)])
        a_qk(0, 0, 0)
        def a_body(j, carry):
            r0, c0 = a_idx(j)
            m = l = acc = None
            for c in range(nch):
                if c + 1 < nch: a_qk(j, c + 1, (c + 1) % 2)
                else: a_qk(jnp.minimum(j + 1, nblk - 1), 0, (c + 1) % 2)
                s = s_ref[c % 2]
                mc = jnp.max(s, axis=0, keepdims=True)
                if c == 0:
                    m = mc
                    p = jnp.exp2(s - m)
                    l = jnp.sum(p, axis=0, keepdims=True)
                    acc = dot_nn(vta[:, c*KC:(c+1)*KC], p.astype(bf16))
                else:
                    mn = jnp.maximum(m, mc)
                    alpha = jnp.exp2(m - mn)
                    p = jnp.exp2(s - mn)
                    l = l * alpha + jnp.sum(p, axis=0, keepdims=True)
                    acc = acc * alpha + dot_nn(vta[:, c*KC:(c+1)*KC], p.astype(bf16))
                    m = mn
            ota[pl.ds(r0, DH), pl.ds(c0, CB)] = (acc / l).astype(bf16)
            return carry
        lax.fori_loop(0, nblk, a_body, 0)

        def ocp(c, half):
            return pltpu.make_async_copy(outv.at[pl.ds(c * RC, RC), pl.ds(half * D, D)],
                                         out_hbm.at[pl.ds(c * RC, RC), pl.ds(half * D, D)], osem.at[half * NRC + c])
        c_awo.wait()
        for c in range(NRC):
            outv[c*RC:(c+1)*RC, 0:D] = dot_tn(ota[:, c*RC:(c+1)*RC], awo[...]).astype(bf16)
            ocp(c, 0).start()

        c_wqkv.wait(); c_xb.wait()
        for c in range(NRC):
            x = xb[c*RC:(c+1)*RC, :]
            qt = (dot_tt(wqkv[:, 0:D], x) * SCALE).astype(bf16)
            for h in range(H):
                for ii in range(RC // QB):
                    i = c * (RC // QB) + ii
                    col = (i * 4 + h % 4) * QB
                    qbd[h*DH:(h+1)*DH, col:col+QB] = qt[h*DH:(h+1)*DH, ii*QB:(ii+1)*QB]
            kb[W + c*RC: W + (c+1)*RC, :] = dot_nn(x, wqkv[:, D:2*D]).astype(bf16)
            vtb[:, W + c*RC: W + (c+1)*RC] = dot_tt(wqkv[:, 2*D:3*D], x).astype(bf16)

        r = lax.broadcasted_iota(jnp.int32, (QB, 4 * QB), 0)
        cq = lax.broadcasted_iota(jnp.int32, (QB, 4 * QB), 1) % QB
        def b_qk(i, g, c, slot):
            k0 = pl.multiple_of(i * QB + CH[c] * QB, QB)
            kg = kb[pl.ds(k0, QB), g*128:(g+1)*128]
            wbd = qbd[g*128:(g+1)*128, pl.ds(pl.multiple_of(i * 4 * QB, 4 * QB), 4 * QB)]
            s_ref[slot] = dot_nn(kg, wbd)
        b_qk(0, 0, 0, 0)
        def b_steps(i, first):
            q0 = pl.multiple_of(i * QB, QB)
            t = 0
            for g in range(NG):
                m = l = acc = None
                for c in range(3):
                    if c + 1 < 3: b_qk(i, g, c + 1, (t + 1) % 2)
                    elif g + 1 < NG: b_qk(i, g + 1, 0, (t + 1) % 2)
                    else: b_qk(jnp.minimum(i + 1, NQ - 1), 0, 0, (t + 1) % 2)
                    s = s_ref[t % 2]
                    if c == 0: s = jnp.where(r <= cq, s, NEG)
                    if c == 2: s = jnp.where(r > cq, s, NEG)
                    if first and c > 0:
                        s = jnp.where(r >= W - CH[c] * QB - q0, s, NEG)
                    mc = jnp.max(s, axis=0, keepdims=True)
                    k0 = pl.multiple_of(i * QB + CH[c] * QB, QB)
                    def pvdot(p):
                        return jnp.concatenate([dot_nn(vtb[(g*4+hh)*DH:(g*4+hh+1)*DH, pl.ds(k0, QB)],
                                                       p[:, hh*QB:(hh+1)*QB].astype(bf16)) for hh in range(4)], axis=1)
                    if c == 0:
                        m = mc
                        p = jnp.exp2(s - m)
                        l = jnp.sum(p, axis=0, keepdims=True)
                        acc = pvdot(p)
                    else:
                        mn = jnp.maximum(m, mc)
                        alpha = jnp.exp2(m - mn)
                        p = jnp.exp2(s - mn)
                        l = l * alpha + jnp.sum(p, axis=0, keepdims=True)
                        acc = acc * alpha + pvdot(p)
                        m = mn
                    t += 1
                o = (acc / l).astype(bf16)
                for hh in range(4):
                    h = g * 4 + hh
                    otb[h*DH:(h+1)*DH, pl.ds(q0, QB)] = o[:, hh*QB:(hh+1)*QB]
        def b_first(i, carry):
            b_steps(i, True); return carry
        def b_body(i, carry):
            b_steps(i, False); return carry
        lax.fori_loop(0, 2, b_first, 0)
        lax.fori_loop(2, NQ, b_body, 0)

        c_bwo.wait()
        for c in range(NRC):
            outv[c*RC:(c+1)*RC, D:2*D] = dot_tn(otb[:, c*RC:(c+1)*RC], bwo[...]).astype(bf16)
            ocp(c, 1).start()
        for half in range(2):
            for c in range(NRC):
                ocp(c, half).wait()

    def f(A_x, A_wq, A_wk, A_wv, A_wo, B_x, B_wqkv, B_wo):
        anyspec = pl.BlockSpec(memory_space=pl.ANY)
        out = pl.pallas_call(
            kernel,
            out_shape=jax.ShapeDtypeStruct((S, 2 * D), bf16),
            in_specs=[anyspec] * 8, out_specs=anyspec,
            scratch_shapes=[
                pltpu.VMEM((S, D), bf16), pltpu.VMEM((D, D), bf16), pltpu.VMEM((DH, D), bf16), pltpu.VMEM((DH, D), bf16),
                pltpu.VMEM((D, D), bf16), pltpu.VMEM((S, D), bf16), pltpu.VMEM((D, 3 * D), bf16), pltpu.VMEM((D, D), bf16),
                pltpu.VMEM((S, DH), bf16), pltpu.VMEM((DH, S), bf16), pltpu.VMEM((D, S), bf16), pltpu.VMEM((D, S), bf16),
                pltpu.VMEM((D, 4 * S), bf16), pltpu.VMEM((S + W, D), bf16), pltpu.VMEM((D, S + W), bf16), pltpu.VMEM((D, S), bf16),
                pltpu.VMEM((2, KC, CB), f32), pltpu.VMEM((S, 2 * D), bf16),
                pltpu.SemaphoreType.DMA((11,)), pltpu.SemaphoreType.DMA((2 * NRC,)),
            ],
            compiler_params=pltpu.CompilerParams(vmem_limit_bytes=120 * 1024 * 1024),
        )(A_x.reshape(S, D), A_wq, A_wk.T, A_wv.T, A_wo, B_x.reshape(S, D), B_wqkv, B_wo)
        return out.reshape(1, S, 2 * D)
    return f


_impl = _make()


@jax.jit
def pallas_concat_heads__grouped_kv_mqa__sliding_block__prompt_kernel(
    A_x: jax.Array,
    A_wq: jax.Array,
    A_wk: jax.Array,
    A_wv: jax.Array,
    A_wo: jax.Array,
    B_x: jax.Array,
    B_wqkv: jax.Array,
    B_wo: jax.Array,
):
    return _impl(A_x, A_wq, A_wk, A_wv, A_wo, B_x, B_wqkv, B_wo)
```

```python
import functools
import jax, jax.numpy as jnp
from jax import lax
from jax.experimental import pallas as pl
from jax.experimental.pallas import tpu as pltpu

S = 2048; D = 1024; H = 32; DH = 32; W = 256
LOG2E = 1.4426950408889634
SCALE = (DH ** -0.5) * LOG2E
f32 = jnp.float32; bf16 = jnp.bfloat16
NEG = -1e30
RC = 512
NRC = S // RC
CB = 512; KC = 128
QB = 128; NG = H // 4; NQ = S // QB
CH = (2, 1, 0)
NB = 4
SW = 256

def dot_tt(w, x): return lax.dot_general(w, x, (((0,), (1,)), ((), ())), preferred_element_type=f32)
def dot_nt(a, b): return lax.dot_general(a, b, (((1,), (1,)), ((), ())), preferred_element_type=f32)
def dot_tn(a, b): return lax.dot_general(a, b, (((0,), (0,)), ((), ())), preferred_element_type=f32)
def dot_nn(a, b): return jnp.dot(a, b, preferred_element_type=f32)

def _make(NA=1, NB_=1, UA=4, UB=1, DA=3, DB=2):
    def kernel(ax_hbm, wq_hbm, wkt_hbm, wvt_hbm, awo_hbm, bx_hbm, wqkv_hbm, bwo_hbm, out_hbm,
               xa, wq, wkt, wvt, awo, xb, wqkv, bwo,
               ka, vta, qta, ota, qbd, kb, vtb, otb, s_ref, outv, isem, osem):
        def cp(src, dst, i): return pltpu.make_async_copy(src, dst, isem.at[i])
        c_wk = cp(wkt_hbm, wkt, 0); c_wv = cp(wvt_hbm, wvt, 1); c_wq = cp(wq_hbm, wq, 2)
        c_xa = [cp(ax_hbm.at[pl.ds(c * RC, RC), :], xa.at[pl.ds(c * RC, RC), :], 3 + c) for c in range(NRC)]
        c_awo = cp(awo_hbm, awo, 7); c_wqkv = cp(wqkv_hbm, wqkv, 8); c_xb = cp(bx_hbm, xb, 9); c_bwo = cp(bwo_hbm, bwo, 10)
        c_wk.start(); c_wv.start(); c_xa[0].start(); c_wq.start()
        for c in range(1, NRC): c_xa[c].start()
        def zbody(i, carry):
            qbd[pl.ds(pl.multiple_of(i * 128, 128), 128), :] = jnp.zeros((128, 4 * S), bf16)
            return carry
        lax.fori_loop(0, D // 128, zbody, 0)
        vtb[:, 0:W] = jnp.zeros((D, W), bf16)
        kb[0:W, :] = jnp.zeros((W, D), bf16)
        c_wk.wait(); c_wv.wait()
        for c in range(NRC):
            c_xa[c].wait()
            if c == 0:
                c_wq.wait()
                c_wqkv.start(); c_xb.start(); c_awo.start(); c_bwo.start()
            x = xa[c*RC:(c+1)*RC, :]
            ka[c*RC:(c+1)*RC, :] = dot_nt(x, wkt[...]).astype(bf16)
            vta[:, c*RC:(c+1)*RC] = dot_nt(wvt[...], x).astype(bf16)
            qta[:, c*RC:(c+1)*RC] = (dot_tt(wq[...], x) * SCALE).astype(bf16)

        nqb = S // CB; nch = S // KC; nblk = H * nqb
        def a_idx(j):
            return pl.multiple_of((j // nqb) * DH, DH), pl.multiple_of((j % nqb) * CB, CB)
        def a_qk(j, c):
            if c >= nch:
                j = jnp.minimum(j + 1, nblk - 1)
            r0, c0 = a_idx(j)
            cc = c % nch
            s_ref[c % NB] = dot_nn(ka[cc*KC:(cc+1)*KC, :], qta[pl.ds(r0, DH), pl.ds(c0, CB)])
        for d in range(DA): a_qk(0, d)
        def a_body(j, carry):
            r0, c0 = a_idx(j)
            m = [None, None]; l = [None, None]; acc = [None, None]
            for c in range(nch):
                for sp in range(2):
                    if sp == 1: a_qk(j, c + DA)
                    s = s_ref[c % NB, :, sp*SW:(sp+1)*SW]
                    mc = jnp.max(s, axis=0, keepdims=True)
                    if c == 0:
                        m[sp] = mc
                        p = jnp.exp2(s - mc)
                        l[sp] = jnp.sum(p, axis=0, keepdims=True)
                        acc[sp] = dot_nn(vta[:, c*KC:(c+1)*KC], p.astype(bf16))
                    else:
                        mn = jnp.maximum(m[sp], mc)
                        alpha = jnp.exp2(m[sp] - mn)
                        p = jnp.exp2(s - mn)
                        l[sp] = l[sp] * alpha + jnp.sum(p, axis=0, keepdims=True)
                        acc[sp] = acc[sp] * alpha + dot_nn(vta[:, c*KC:(c+1)*KC], p.astype(bf16))
                        m[sp] = mn
            for sp in range(2):
                ota[pl.ds(r0, DH), pl.ds(c0 + sp * SW, SW)] = (acc[sp] / l[sp]).astype(bf16)
            return carry
        lax.fori_loop(0, nblk * NA, a_body, 0, unroll=UA)

        def ocp(c, half):
            return pltpu.make_async_copy(outv.at[pl.ds(c * RC, RC), pl.ds(half * D, D)],
                                         out_hbm.at[pl.ds(c * RC, RC), pl.ds(half * D, D)], osem.at[half * NRC + c])
        c_awo.wait()
        for c in range(NRC):
            outv[c*RC:(c+1)*RC, 0:D] = dot_tn(ota[:, c*RC:(c+1)*RC], awo[...]).astype(bf16)
            ocp(c, 0).start()

        c_wqkv.wait(); c_xb.wait()
        for c in range(NRC):
            x = xb[c*RC:(c+1)*RC, :]
            qt = (dot_tt(wqkv[:, 0:D], x) * SCALE).astype(bf16)
            for h in range(H):
                for ii in range(RC // QB):
                    i = c * (RC // QB) + ii
                    col = (i * 4 + h % 4) * QB
                    qbd[h*DH:(h+1)*DH, col:col+QB] = qt[h*DH:(h+1)*DH, ii*QB:(ii+1)*QB]
            kb[W + c*RC: W + (c+1)*RC, :] = dot_nn(x, wqkv[:, D:2*D]).astype(bf16)
            vtb[:, W + c*RC: W + (c+1)*RC] = dot_tt(wqkv[:, 2*D:3*D], x).astype(bf16)

        NT = NG * 3
        r = lax.broadcasted_iota(jnp.int32, (QB, SW), 0)
        cq = lax.broadcasted_iota(jnp.int32, (QB, SW), 1) % QB
        def b_qk(i, t):
            if t >= NT:
                i = jnp.minimum(i + 1, NQ - 1)
            tt = t % NT
            g, c = tt // 3, tt % 3
            k0 = pl.multiple_of(i * QB + CH[c] * QB, QB)
            kg = kb[pl.ds(k0, QB), g*128:(g+1)*128]
            wbd = qbd[g*128:(g+1)*128, pl.ds(pl.multiple_of(i * 4 * QB, 4 * QB), 4 * QB)]
            s_ref[t % NB] = dot_nn(kg, wbd)
        for d in range(DB): b_qk(0, d)
        def b_steps(i, first):
            q0 = pl.multiple_of(i * QB, QB)
            for g in range(NG):
                m = [None, None]; l = [None, None]; acc = [None, None]
                for c in range(3):
                    t = g * 3 + c
                    k0 = pl.multiple_of(i * QB + CH[c] * QB, QB)
                    for sp in range(2):
                        if sp == 1: b_qk(i, t + DB)
                        s = s_ref[t % NB, :, sp*SW:(sp+1)*SW]
                        if c == 0: s = jnp.where(r <= cq, s, NEG)
                        if c == 2: s = jnp.where(r > cq, s, NEG)
                        if first and c > 0:
                            s = jnp.where(r >= W - CH[c] * QB - q0, s, NEG)
                        mc = jnp.max(s, axis=0, keepdims=True)
                        def pvdot(p):
                            return jnp.concatenate([dot_nn(vtb[(g*4+sp*2+hh)*DH:(g*4+sp*2+hh+1)*DH, pl.ds(k0, QB)],
                                                           p[:, hh*QB:(hh+1)*QB].astype(bf16)) for hh in range(2)], axis=1)
                        if c == 0:
                            m[sp] = mc
                            p = jnp.exp2(s - mc)
                            l[sp] = jnp.sum(p, axis=0, keepdims=True)
                            acc[sp] = pvdot(p)
                        else:
                            mn = jnp.maximum(m[sp], mc)
                            alpha = jnp.exp2(m[sp] - mn)
                            p = jnp.exp2(s - mn)
                            l[sp] = l[sp] * alpha + jnp.sum(p, axis=0, keepdims=True)
                            acc[sp] = acc[sp] * alpha + pvdot(p)
                            m[sp] = mn
                for sp in range(2):
                    o = (acc[sp] / l[sp]).astype(bf16)
                    for hh in range(2):
                        h = g * 4 + sp * 2 + hh
                        otb[h*DH:(h+1)*DH, pl.ds(q0, QB)] = o[:, hh*QB:(hh+1)*QB]
        def b_first(i, carry):
            b_steps(i, True); return carry
        def b_body(i, carry):
            b_steps(i, False); return carry
        lax.fori_loop(0, 2 * NB_, b_first, 0)
        lax.fori_loop(2, 2 + (NQ - 2) * NB_, b_body, 0, unroll=UB)

        c_bwo.wait()
        for c in range(NRC):
            outv[c*RC:(c+1)*RC, D:2*D] = dot_tn(otb[:, c*RC:(c+1)*RC], bwo[...]).astype(bf16)
            ocp(c, 1).start()
        for half in range(2):
            for c in range(NRC):
                ocp(c, half).wait()

    def f(A_x, A_wq, A_wk, A_wv, A_wo, B_x, B_wqkv, B_wo):
        anyspec = pl.BlockSpec(memory_space=pl.ANY)
        out = pl.pallas_call(
            kernel,
            out_shape=jax.ShapeDtypeStruct((S, 2 * D), bf16),
            in_specs=[anyspec] * 8, out_specs=anyspec,
            scratch_shapes=[
                pltpu.VMEM((S, D), bf16), pltpu.VMEM((D, D), bf16), pltpu.VMEM((DH, D), bf16), pltpu.VMEM((DH, D), bf16),
                pltpu.VMEM((D, D), bf16), pltpu.VMEM((S, D), bf16), pltpu.VMEM((D, 3 * D), bf16), pltpu.VMEM((D, D), bf16),
                pltpu.VMEM((S, DH), bf16), pltpu.VMEM((DH, S), bf16), pltpu.VMEM((D, S), bf16), pltpu.VMEM((D, S), bf16),
                pltpu.VMEM((D, 4 * S), bf16), pltpu.VMEM((S + W, D), bf16), pltpu.VMEM((D, S + W), bf16), pltpu.VMEM((D, S), bf16),
                pltpu.VMEM((NB, KC, CB), f32), pltpu.VMEM((S, 2 * D), bf16),
                pltpu.SemaphoreType.DMA((11,)), pltpu.SemaphoreType.DMA((2 * NRC,)),
            ],
            compiler_params=pltpu.CompilerParams(vmem_limit_bytes=120 * 1024 * 1024),
        )(A_x.reshape(S, D), A_wq, A_wk.T, A_wv.T, A_wo, B_x.reshape(S, D), B_wqkv, B_wo)
        return out.reshape(1, S, 2 * D)
    return f


_impl = _make()


@jax.jit
def pallas_concat_heads__grouped_kv_mqa__sliding_block__prompt_kernel(
    A_x: jax.Array,
    A_wq: jax.Array,
    A_wk: jax.Array,
    A_wv: jax.Array,
    A_wo: jax.Array,
    B_x: jax.Array,
    B_wqkv: jax.Array,
    B_wo: jax.Array,
):
    return _impl(A_x, A_wq, A_wk, A_wv, A_wo, B_x, B_wqkv, B_wo)
```

```python
import jax
import jax.numpy as jnp
from jax import lax
from jax.experimental import pallas as pl
from jax.experimental.pallas import tpu as pltpu

S = 2048; D = 1024; H = 32; DH = 32; W = 256
LOG2E = 1.4426950408889634
SCALE = (DH ** -0.5) * LOG2E
f32 = jnp.float32; bf16 = jnp.bfloat16
NEG = -1e30
RC = 512
NRC = S // RC
CB = 512; KC = 128
QB = 128; NG = H // 4; NQ = S // QB
NB = 4
SW = 256
DA = 3; DB = 2
UA = 8
PIECES = (1024, 512, 256, 128, 128)


def _dot_tt(w, x):
    return lax.dot_general(w, x, (((0,), (1,)), ((), ())), preferred_element_type=f32)


def _dot_nt(a, b):
    return lax.dot_general(a, b, (((1,), (1,)), ((), ())), preferred_element_type=f32)


def _dot_tn(a, b):
    return lax.dot_general(a, b, (((0,), (0,)), ((), ())), preferred_element_type=f32)


def _dot_nn(a, b):
    return jnp.dot(a, b, preferred_element_type=f32)


def _kernel(ax_hbm, wq_hbm, wkt_hbm, wvt_hbm, awo_hbm, bx_hbm, wqkv_hbm, bwo_hbm, out_hbm,
            xa, wq, wkt, wvt, awo, xb, wqkv, bwo,
            ka, vta, qta, ota, qbd, kb, vtb, otb, s_ref, outv, isem, osem):
    def cp(src, dst, i):
        return pltpu.make_async_copy(src, dst, isem.at[i])
    c_wk = cp(wkt_hbm, wkt, 0); c_wv = cp(wvt_hbm, wvt, 1); c_wq = cp(wq_hbm, wq, 2)
    c_xa = [cp(ax_hbm.at[pl.ds(c * RC, RC), :], xa.at[pl.ds(c * RC, RC), :], 3 + c) for c in range(NRC)]
    c_awo = cp(awo_hbm, awo, 7); c_wqkv = cp(wqkv_hbm, wqkv, 8)
    c_xb = cp(bx_hbm, xb, 9); c_bwo = cp(bwo_hbm, bwo, 10)
    c_wk.start(); c_wv.start(); c_xa[0].start(); c_wq.start()

    def zbody(i, carry):
        qbd[pl.ds(pl.multiple_of(i * 128, 128), 128), :] = jnp.zeros((128, 4 * S), bf16)
        return carry
    lax.fori_loop(0, D // 128, zbody, 0)
    c_wk.wait(); c_wv.wait()

    for c in range(NRC):
        c_xa[c].wait()
        if c == 0:
            for cc in range(1, NRC):
                c_xa[cc].start()
            c_wq.wait()
            c_wqkv.start(); c_xb.start(); c_awo.start(); c_bwo.start()
        x = xa[c*RC:(c+1)*RC, :]
        ka[c*RC:(c+1)*RC, :] = _dot_nt(x, wkt[...]).astype(bf16)
        vta[:, c*RC:(c+1)*RC] = _dot_nt(wvt[...], x).astype(bf16)
        qta[:, c*RC:(c+1)*RC] = (_dot_tt(wq[...], x) * SCALE).astype(bf16)

    nqb = S // CB; nch = S // KC; nblk = H * nqb

    def a_idx(j):
        return pl.multiple_of((j // nqb) * DH, DH), pl.multiple_of((j % nqb) * CB, CB)

    def a_qk(j, c):
        if c >= nch:
            j = jnp.minimum(j + 1, nblk - 1)
        r0, c0 = a_idx(j)
        cc = c % nch
        s_ref[c % NB] = _dot_nn(ka[cc*KC:(cc+1)*KC, :], qta[pl.ds(r0, DH), pl.ds(c0, CB)])

    for d in range(DA):
        a_qk(0, d)

    def a_body(j, carry):
        r0, c0 = a_idx(j)
        m = [None, None]; l = [None, None]; acc = [None, None]
        for c in range(nch):
            for sp in range(2):
                if sp == 1:
                    a_qk(j, c + DA)
                s = s_ref[c % NB, :, sp*SW:(sp+1)*SW]
                mc = jnp.max(s, axis=0, keepdims=True)
                if c == 0:
                    m[sp] = mc
                    p = jnp.exp2(s - mc)
                    l[sp] = jnp.sum(p, axis=0, keepdims=True)
                    acc[sp] = _dot_nn(vta[:, c*KC:(c+1)*KC], p.astype(bf16))
                else:
                    mn = jnp.maximum(m[sp], mc)
                    alpha = jnp.exp2(m[sp] - mn)
                    p = jnp.exp2(s - mn)
                    l[sp] = l[sp] * alpha + jnp.sum(p, axis=0, keepdims=True)
                    acc[sp] = acc[sp] * alpha + _dot_nn(vta[:, c*KC:(c+1)*KC], p.astype(bf16))
                    m[sp] = mn
        for sp in range(2):
            ota[pl.ds(r0, DH), pl.ds(c0 + sp * SW, SW)] = (acc[sp] / l[sp]).astype(bf16)
        return carry
    lax.fori_loop(0, nblk, a_body, 0, unroll=UA)

    def ocp_a(c):
        return pltpu.make_async_copy(outv.at[pl.ds(c * RC, RC), pl.ds(0, D)],
                                     out_hbm.at[pl.ds(c * RC, RC), pl.ds(0, D)], osem.at[c])
    c_awo.wait()
    for c in range(NRC):
        outv[c*RC:(c+1)*RC, 0:D] = _dot_tn(ota[:, c*RC:(c+1)*RC], awo[...]).astype(bf16)
        ocp_a(c).start()

    c_wqkv.wait(); c_xb.wait()
    for c in range(NRC):
        x = xb[c*RC:(c+1)*RC, :]
        qt = (_dot_tt(wqkv[:, 0:D], x) * SCALE).astype(bf16)
        for h in range(H):
            for ii in range(RC // QB):
                i = c * (RC // QB) + ii
                col = (i * 4 + h % 4) * QB
                qbd[h*DH:(h+1)*DH, col:col+QB] = qt[h*DH:(h+1)*DH, ii*QB:(ii+1)*QB]
        kb[c*RC:(c+1)*RC, :] = _dot_nn(x, wqkv[:, D:2*D]).astype(bf16)
        vtb[:, c*RC:(c+1)*RC] = _dot_tt(wqkv[:, 2*D:3*D], x).astype(bf16)

    NT = NG * 3
    r = lax.broadcasted_iota(jnp.int32, (QB, SW), 0)
    cq = lax.broadcasted_iota(jnp.int32, (QB, SW), 1) % QB
    pro = [(i, g, c) for i in range(2) for g in range(NG) for c in range(i + 1)]

    def b_qk(i, g, c, slot):
        if isinstance(i, int):
            kg = kb[(i-c)*QB:(i-c+1)*QB, g*128:(g+1)*128]
            wbd = qbd[g*128:(g+1)*128, i*4*QB:(i+1)*4*QB]
        else:
            k0 = pl.multiple_of((i - c) * QB, QB)
            kg = kb[pl.ds(k0, QB), g*128:(g+1)*128]
            wbd = qbd[g*128:(g+1)*128, pl.ds(pl.multiple_of(i * 4 * QB, 4 * QB), 4 * QB)]
        s_ref[slot] = _dot_nn(kg, wbd)

    def b_group(i, g, nc, t0, prefetch):
        static = isinstance(i, int)
        m = [None, None]; l = [None, None]; acc = [None, None]
        for c in range(nc):
            t = t0 + c
            for sp in range(2):
                if sp == 1:
                    prefetch(t + DB)
                s = s_ref[t % NB, :, sp*SW:(sp+1)*SW]
                if c == 0:
                    s = jnp.where(r <= cq, s, NEG)
                if c == 2:
                    s = jnp.where(r > cq, s, NEG)
                mc = jnp.max(s, axis=0, keepdims=True)

                def pvdot(p):
                    outs = []
                    for hh in range(2):
                        h = g * 4 + sp * 2 + hh
                        if static:
                            vt = vtb[h*DH:(h+1)*DH, (i-c)*QB:(i-c+1)*QB]
                        else:
                            vt = vtb[h*DH:(h+1)*DH, pl.ds(pl.multiple_of((i - c) * QB, QB), QB)]
                        outs.append(_dot_nn(vt, p[:, hh*QB:(hh+1)*QB].astype(bf16)))
                    return jnp.concatenate(outs, axis=1)
                if c == 0:
                    m[sp] = mc
                    p = jnp.exp2(s - mc)
                    l[sp] = jnp.sum(p, axis=0, keepdims=True)
                    acc[sp] = pvdot(p)
                else:
                    mn = jnp.maximum(m[sp], mc)
                    alpha = jnp.exp2(m[sp] - mn)
                    p = jnp.exp2(s - mn)
                    l[sp] = l[sp] * alpha + jnp.sum(p, axis=0, keepdims=True)
                    acc[sp] = acc[sp] * alpha + pvdot(p)
                    m[sp] = mn
        for sp in range(2):
            o = (acc[sp] / l[sp]).astype(bf16)
            for hh in range(2):
                h = g * 4 + sp * 2 + hh
                if static:
                    otb[h*DH:(h+1)*DH, i*QB:(i+1)*QB] = o[:, hh*QB:(hh+1)*QB]
                else:
                    otb[h*DH:(h+1)*DH, pl.ds(pl.multiple_of(i * QB, QB), QB)] = o[:, hh*QB:(hh+1)*QB]

    def pro_prefetch(t):
        if t < len(pro):
            i, g, c = pro[t]
        else:
            tt = t - len(pro)
            i, g, c = 2, tt // 3, tt % 3
        b_qk(i, g, c, t % NB)

    for d in range(DB):
        pro_prefetch(d)
    t0 = 0
    for i in range(2):
        for g in range(NG):
            b_group(i, g, i + 1, t0, pro_prefetch)
            t0 += i + 1

    def b_body(i, carry):
        def prefetch(t):
            ii = i if t < NT else jnp.minimum(i + 1, NQ - 1)
            tt = t % NT
            b_qk(ii, tt // 3, tt % 3, t % NB)
        for g in range(NG):
            b_group(i, g, 3, g * 3, prefetch)
        return carry
    lax.fori_loop(2, NQ, b_body, 0)

    c_bwo.wait()
    ocs = []
    r0 = 0
    for n, pr in enumerate(PIECES):
        outv[r0:r0+pr, D:2*D] = _dot_tn(otb[:, r0:r0+pr], bwo[...]).astype(bf16)
        oc = pltpu.make_async_copy(outv.at[pl.ds(r0, pr), pl.ds(D, D)],
                                   out_hbm.at[pl.ds(r0, pr), pl.ds(D, D)], osem.at[NRC + n])
        oc.start()
        ocs.append(oc)
        r0 += pr
    for c in range(NRC):
        ocp_a(c).wait()
    for oc in ocs:
        oc.wait()


@jax.jit
def pallas_concat_heads__grouped_kv_mqa__sliding_block__prompt_kernel(
    A_x: jax.Array,
    A_wq: jax.Array,
    A_wk: jax.Array,
    A_wv: jax.Array,
    A_wo: jax.Array,
    B_x: jax.Array,
    B_wqkv: jax.Array,
    B_wo: jax.Array,
):
    anyspec = pl.BlockSpec(memory_space=pl.ANY)
    out = pl.pallas_call(
        _kernel,
        out_shape=jax.ShapeDtypeStruct((S, 2 * D), bf16),
        in_specs=[anyspec] * 8,
        out_specs=anyspec,
        scratch_shapes=[
            pltpu.VMEM((S, D), bf16), pltpu.VMEM((D, D), bf16), pltpu.VMEM((DH, D), bf16),
            pltpu.VMEM((DH, D), bf16), pltpu.VMEM((D, D), bf16), pltpu.VMEM((S, D), bf16),
            pltpu.VMEM((D, 3 * D), bf16), pltpu.VMEM((D, D), bf16),
            pltpu.VMEM((S, DH), bf16), pltpu.VMEM((DH, S), bf16),
            pltpu.VMEM((D, S), bf16), pltpu.VMEM((D, S), bf16),
            pltpu.VMEM((D, 4 * S), bf16), pltpu.VMEM((S, D), bf16),
            pltpu.VMEM((D, S), bf16), pltpu.VMEM((D, S), bf16),
            pltpu.VMEM((NB, KC, CB), f32), pltpu.VMEM((S, 2 * D), bf16),
            pltpu.SemaphoreType.DMA((11,)), pltpu.SemaphoreType.DMA((NRC + len(PIECES),)),
        ],
        compiler_params=pltpu.CompilerParams(vmem_limit_bytes=120 * 1024 * 1024),
    )(A_x.reshape(S, D), A_wq, A_wk.T, A_wv.T, A_wo, B_x.reshape(S, D), B_wqkv, B_wo)
    return out.reshape(1, S, 2 * D)
```
